```python
import jax
import jax.numpy as jnp

def _softmax(x, axis=-1):
    return jax.nn.softmax(x, axis=axis)
def _gelu(x):
    return jax.nn.gelu(x, approximate=True)
def _silu(x):
    return jax.nn.silu(x)
def _sigmoid(x):
    return jax.nn.sigmoid(x)
def _layernorm(x, axis=-1, eps=1e-5):
    m = jnp.mean(x, axis=axis, keepdims=True)
    v = jnp.var(x, axis=axis, keepdims=True)
    return (x - m) / jnp.sqrt(v + eps)
def _scatter_add(tgt, idx, src, axis=0):
    return tgt.at[idx].add(src)
def _segment_sum(src, seg, n):
    return jax.ops.segment_sum(src, seg, n)
class _Rng:
    def __init__(self, key):
        self._k = key
    def _next(self):
        self._k, sub = jax.random.split(self._k)
        return sub
    def normal(self, shape):
        return jax.random.normal(self._next(), shape, dtype=jnp.bfloat16)
    def randint(self, lo, hi, shape):
        return jax.random.randint(self._next(), shape, lo, hi, dtype=jnp.int32)
    def uniform(self, shape, lo=0.0, hi=1.0):
        return jax.random.uniform(self._next(), shape, jnp.bfloat16, lo, hi)
    def permutation(self, n):
        return jax.random.permutation(self._next(), n)


kernel_name = 'sequential_preLN__sliding_block_cached__moe_arch_mod__decode'

def setup_inputs():
    _rng = _Rng(jax.random.key(int.from_bytes(__import__("os").urandom(4), "little")))
    _w = (lambda a: (lambda t: t.astype(jnp.bfloat16) if jnp.issubdtype(t.dtype, jnp.floating) else t)(jnp.asarray(a)))
    def _A_setup():
        B, Sq, D = 1, 1, 640
        Hq, Hkv, Sk, Dh = 32, 32, 32768, 192
        assert Hq % Hkv == 0, (Hq, Hkv)
        return {
            "x": _w((lambda *s: _rng.normal(s) * 0.05)(B, Sq, D)),
            "k_cache": _w((lambda *s: _rng.normal(s) * 0.05)(B, Hkv, Sk, Dh)),
            "v_cache": _w((lambda *s: _rng.normal(s) * 0.05)(B, Hkv, Sk, Dh)),
            "wq": _w((lambda *s: _rng.normal(s) * 0.05)(D, Hq * Dh) * (D ** -0.5)),
            "wo": _w((lambda *s: _rng.normal(s) * 0.05)(Hq * Dh, D) * ((Hq * Dh) ** -0.5)),
        }
    _A_in = _A_setup()

    def _B_setup():
        B, S, D, F, C = 1, 1, 640, 1536, 1
        return {
            "x": _w((lambda *s: _rng.normal(s) * 0.05)(B, S, D)),
            "w_r": _w((lambda *s: _rng.normal(s) * 0.05)(D)),
            "w_gate": _w((lambda *s: _rng.normal(s) * 0.05)(D, F)),
            "w_up": _w((lambda *s: _rng.normal(s) * 0.05)(D, F)),
            "w_down": _w((lambda *s: _rng.normal(s) * 0.05)(F, D)),
        }
    _B_in = _B_setup()

    return {
        "A_x": _A_in["x"],
        "A_k_cache": _A_in["k_cache"],
        "A_v_cache": _A_in["v_cache"],
        "A_wq": _A_in["wq"],
        "A_wo": _A_in["wo"],
        "B_x": _B_in["x"],
        "B_w_r": _B_in["w_r"],
        "B_w_gate": _B_in["w_gate"],
        "B_w_up": _B_in["w_up"],
        "B_w_down": _B_in["w_down"],
    }

def reference(A_x, A_k_cache, A_v_cache, A_wq, A_wo, B_x, B_w_r, B_w_gate, B_w_up, B_w_down):
    def _A_ref(x, k_cache, v_cache, wq, wo):
        B, Sq, D = x.shape
        Hq, Dh = 32, 192
        Hkv, Sk = k_cache.shape[1], k_cache.shape[2]
        W = min(4096, max(256, Sk // 4))
        rep = Hq // Hkv
        q = (lambda x, *d: x.transpose(*d))((x @ wq).reshape(B, Sq, Hq, Dh), 0, 2, 1, 3)
        k = jnp.repeat(k_cache[:, :, Sk - W:, :], rep, axis=1)
        v = jnp.repeat(v_cache[:, :, Sk - W:, :], rep, axis=1)
        scores = jnp.einsum("bhqd,bhkd->bhqk", q, k) * (Dh ** -0.5)
        p = _softmax(scores, axis=-1)
        o = jnp.einsum("bhqk,bhkd->bhqd", p, v)
        return (lambda x, *d: x.transpose(*d))(o, 0, 2, 1, 3).reshape(B, Sq, Hq * Dh) @ wo

    def _B_ref(x, w_r, w_gate, w_up, w_down):
        B, S, D = x.shape
        C = 1
        r = x @ w_r
        idx = jnp.argsort(-r, axis=-1)[:, :C]
        idx_e = jnp.repeat(idx.reshape(B, C, 1), D, axis=2)
        x_sel = jnp.take_along_axis(x, idx_e, axis=1)
        g = _silu(x_sel @ w_gate)
        u = x_sel @ w_up
        y = (g * u) @ w_down
        r_sel = _sigmoid(jnp.take_along_axis(r, idx, axis=1))
        y = y * r_sel.reshape(B, C, 1)
        b_off = (jnp.arange(B) * S).reshape(B, 1)
        flat_idx = (idx + b_off).reshape(B * C)
        zero = (x * 0.0).reshape(B * S, D)
        upd = _scatter_add(zero, flat_idx, y.reshape(B * C, D), axis=0)
        return x + upd.reshape(B, S, D)

    x = A_x
    h = x + _A_ref(_layernorm(x, axis=-1), A_k_cache, A_v_cache, A_wq, A_wo)
    h2 = h + _B_ref(_layernorm(h, axis=-1), B_w_r, B_w_gate, B_w_up, B_w_down)
    return h2
```

```python
import jax
import jax.numpy as jnp
from jax import lax
import jax.experimental.pallas as pl
import jax.experimental.pallas.tpu as pltpu

EPS = 1e-5
BLK = 128
NBUF = 3
STRIDE_Q, STRIDE_O, STRIDE_FFN = 8, 20, 5
DOWN_GROUPS = (32, 16, 8, 4)
QUEUE_LAG = 24

f32, bf16 = jnp.float32, jnp.bfloat16


def _tile_order(w):
    r, c = w.shape
    return w.reshape(r // 8, 8, c // 128, 128).transpose(0, 2, 1, 3).reshape(r * c // 128, 128)


def _layernorm(x):
    m = jnp.mean(x, axis=-1, keepdims=True)
    d = x - m
    v = jnp.mean(d * d, axis=-1, keepdims=True)
    return d / jnp.sqrt(v + EPS)


def _kernel(x_hbm, k_hbm, v_hbm, wq_hbm, wo_hbm, wr_hbm, wg_hbm, wu_hbm, wd_hbm,
            o_ref,
            x_s, wr_s, wq_s, wo_s, wg_s, wu_s, wd_s, k_s, v_s, q_s, p_s, lhs_s, y_s,
            sem_kv, sem_w, sem_d, *, H, Dh, Sk, W, F):
    D = x_hbm.shape[-1]
    TR = Dh // 8
    ROW_BLKS = Sk // (16 * 128)
    HALVES = W // (16 * 128)
    DT, FT = D // 128, F // 128
    QG = H * Dh // (16 * 128)

    def block(src, src_blk, dst, dst_blk, sem, queue):
        def rows(b):
            return pl.ds(b * BLK if isinstance(b, int) else pl.multiple_of(b * BLK, BLK), BLK)
        pltpu.make_async_copy(src.at[rows(src_blk)], dst.at[rows(dst_blk)], sem).start(priority=queue)

    def done(dst, sem):
        pltpu.make_async_copy(dst, dst, sem).wait()

    def weight_start(src, dst, sem, stride):
        n = src.shape[0] // BLK // stride

        def outer(j, _):
            def inner(i, _):
                for queue in range(2):
                    b = (2 * i + queue) * stride + j
                    block(src, b, dst, b, sem, queue)
            lax.fori_loop(0, n // 2, inner, None)
        lax.fori_loop(0, stride, outer, None)

    def kv_start(h, slot):
        first = h * (TR * ROW_BLKS) + ROW_BLKS - HALVES
        for a, (src, dst) in enumerate(((k_hbm, k_s), (v_hbm, v_s))):
            for hf in (range(HALVES), reversed(range(HALVES)))[a]:
                def body(i, _):
                    for queue in range(2):
                        tr = 2 * i + queue
                        block(src, first + tr * ROW_BLKS + hf, dst.at[slot], hf * TR + tr,
                              sem_kv.at[a, slot], queue)
                lax.fori_loop(0, TR // 2, body, None)

    n_down = wd_hbm.shape[0] // BLK
    per = n_down // STRIDE_FFN
    down_src = [(i % per) * STRIDE_FFN + i // per for i in range(n_down)]
    landing = sorted(range(n_down), key=lambda i: i + QUEUE_LAG * (i % 2))
    down_slot = [landing.index(i) for i in range(n_down)]
    bounds = [sum(DOWN_GROUPS[:g]) for g in range(len(DOWN_GROUPS) + 1)]

    def down_start():
        for i in range(n_down):
            g = max(g for g in range(len(DOWN_GROUPS)) if bounds[g] <= down_slot[i])
            block(wd_hbm, down_src[i], wd_s, down_slot[i], sem_d.at[g], i % 2)

    x_cp = pltpu.make_async_copy(x_hbm, x_s, sem_w.at[0])
    wr_cp = pltpu.make_async_copy(wr_hbm, wr_s, sem_w.at[1])

    weight_start(wq_hbm, wq_s, sem_w.at[2], STRIDE_Q)
    x_cp.start()
    wr_cp.start(priority=1)
    weight_start(wo_hbm, wo_s, sem_w.at[3], STRIDE_O)
    kv_start(0, 0)

    lane = lax.broadcasted_iota(jnp.int32, (8, 128), 1)
    lane16 = lax.broadcasted_iota(jnp.int32, (16, 128), 1)
    row16 = lax.broadcasted_iota(jnp.int32, (16, 128), 0)
    in_tile = lane & 7
    diagonal = (lane16 >> 3) == row16

    def spread(c, vec, idx, keep):
        g = jnp.take_along_axis(jnp.broadcast_to(vec, (8, 128)), idx, axis=1)
        g = jnp.where(keep, jnp.concatenate([g, g], axis=0), 0.0)
        lhs_s[:, c * 128:(c + 1) * 128] = g.astype(bf16)

    def matmul(lo, hi, w):
        return jnp.dot(lhs_s[:, lo * 128:hi * 128], w, preferred_element_type=f32)

    x_cp.wait()
    x = x_s[0].astype(f32)
    xn = _layernorm(x)
    for tr in range(D // 8):
        spread(tr, xn[:, tr // 16 * 128:(tr // 16 + 1) * 128], in_tile + 8 * (tr % 16), diagonal)
    done(wq_s, sem_w.at[2])
    for g in range(QG):
        w = jnp.concatenate([wq_s[(QG * tr + g) * BLK:(QG * tr + g + 1) * BLK] for tr in range(D // 8)], axis=0)
        q_s[16 * g:16 * (g + 1)] = matmul(0, D // 8, w)
    kv_start(1, 1)
    done(wo_s, sem_w.at[3])

    scale = Dh ** -0.5

    def head(h, slot, acc):
        for tr in range(TR):
            f = h * Dh + 8 * tr
            spread(tr, q_s[pl.ds(f >> 7, 1), :], in_tile + (f & 127), diagonal)
        done(k_s.at[slot], sem_kv.at[0, slot])
        s = jnp.concatenate([matmul(0, TR, k_s[slot, hf * TR * BLK:(hf + 1) * TR * BLK])
                             for hf in range(HALVES)], axis=0) * scale
        m = jnp.max(jnp.max(s, axis=0, keepdims=True), axis=1, keepdims=True)
        e = jnp.exp(s - m)
        inv = 1.0 / jnp.sum(jnp.sum(e, axis=0, keepdims=True), axis=1, keepdims=True)
        for j in range(W // 128):
            p_s[j] = jnp.broadcast_to(e[j:j + 1], (8, 128))
        done(v_s.at[slot], sem_kv.at[1, slot])
        acc = list(acc)
        row0 = pl.multiple_of(h * (Dh * DT), 16)
        for t2 in range(TR // 2):
            o = []
            for tr in (2 * t2, 2 * t2 + 1):
                a0 = jnp.zeros((8, 128), f32)
                a1 = jnp.zeros((8, 128), f32)
                for hf in range(HALVES):
                    for j in range(0, 16, 2):
                        r = (hf * TR + tr) * BLK + 8 * j
                        vv = v_s[slot, r:r + 16, :].astype(f32)
                        a0 = a0 + vv[:8] * p_s[hf * 16 + j]
                        a1 = a1 + vv[8:] * p_s[hf * 16 + j + 1]
                o.append(jnp.sum(a0 + a1, axis=-1, keepdims=True) * inv)
            ww = wo_s[pl.ds(row0 + t2 * 16 * DT, 16 * DT), :].astype(f32)
            for t in range(2 * DT):
                acc[t % DT] = acc[t % DT] + ww[8 * t:8 * t + 8] * o[t // DT]
        return tuple(acc)

    def step(h, carry):
        slot, acc = carry

        @pl.when(h < H - 2)
        def _():
            kv_start(h + 2, jnp.where(slot + 2 >= NBUF, slot + 2 - NBUF, slot + 2))

        @pl.when(h == H - 2)
        def _():
            weight_start(wg_hbm, wg_s, sem_w.at[4], STRIDE_FFN)
            weight_start(wu_hbm, wu_s, sem_w.at[5], STRIDE_FFN)

        pl.when(h == H - 1)(down_start)
        return jnp.where(slot + 1 == NBUF, 0, slot + 1), head(h, slot, acc)

    acc = tuple(jnp.zeros((8, 128), f32) for _ in range(DT))
    _, acc = lax.fori_loop(0, H, step, (0, acc))

    hres = x + jnp.concatenate([jnp.sum(a, axis=0, keepdims=True) for a in acc], axis=1)
    hn = _layernorm(hres)
    wr_cp.wait()
    wr = wr_s[...].astype(f32).reshape(1, D)
    gate = jax.nn.sigmoid(jnp.sum(hn * wr, axis=-1, keepdims=True))
    resid = hres + hn

    def spread_for(slot, blk, vec, ct):
        k0 = 8 * (16 * blk // ct)
        t, t16 = 16 * blk % ct + (lane >> 3), 16 * blk % ct + (lane16 >> 3)
        spread(slot, vec(k0 // 128), k0 % 128 + 8 * (t // ct) + in_tile, (t16 % ct) == row16)

    n_up = wg_hbm.shape[0] // BLK
    for b in range(n_up):
        spread_for(b, b, lambda i: hn[:, 128 * i:128 * (i + 1)], FT)
    done(wg_s, sem_w.at[4])
    g = matmul(0, n_up, wg_s[...])
    y_s[...] = g * jax.nn.sigmoid(g)
    done(wu_s, sem_w.at[5])
    gu = y_s[...] * matmul(0, n_up, wu_s[...])
    for i in range(n_down):
        spread_for(down_slot[i], down_src[i], lambda a: gu[a:a + 1], DT)
    y_s[...] = jnp.zeros_like(y_s)
    for g in range(len(DOWN_GROUPS)):
        lo, hi = bounds[g], bounds[g + 1]
        done(wd_s.at[lo * BLK:hi * BLK], sem_d.at[g])
        y = y_s[...] + matmul(lo, hi, wd_s[lo * BLK:hi * BLK])
        if g + 1 < len(DOWN_GROUPS):
            y_s[...] = y
    y = jnp.concatenate([y[i:i + 1] for i in range(DT)], axis=1)
    o_ref[0] = (resid + y * gate).astype(o_ref.dtype)


@jax.jit
def pallas_sequential_preLN__sliding_block_cached__moe_arch_mod__decode_kernel(
    A_x: jax.Array,
    A_k_cache: jax.Array,
    A_v_cache: jax.Array,
    A_wq: jax.Array,
    A_wo: jax.Array,
    B_x: jax.Array,
    B_w_r: jax.Array,
    B_w_gate: jax.Array,
    B_w_up: jax.Array,
    B_w_down: jax.Array,
):
    del B_x
    _, H, Sk, Dh = A_k_cache.shape
    D, F = B_w_gate.shape
    W = min(4096, max(256, Sk // 4))
    k, v = (_tile_order(jnp.transpose(c, (0, 1, 3, 2)).reshape(H * Dh, Sk)) for c in (A_k_cache, A_v_cache))
    wq, wo, wg, wu, wd = (_tile_order(w) for w in (A_wq, A_wo, B_w_gate, B_w_up, B_w_down))

    def like(a):
        return pltpu.VMEM(a.shape, a.dtype)

    def kernel(*refs):
        _kernel(*refs, H=H, Dh=Dh, Sk=Sk, W=W, F=F)

    return pl.pallas_call(
        kernel,
        out_shape=jax.ShapeDtypeStruct(A_x.shape, A_x.dtype),
        in_specs=[pl.BlockSpec(memory_space=pl.ANY)] * 9,
        scratch_shapes=[
            like(A_x), like(B_w_r), like(wq), like(wo), like(wg), like(wu), like(wd),
            pltpu.VMEM((NBUF, Dh * W // 128, 128), k.dtype),
            pltpu.VMEM((NBUF, Dh * W // 128, 128), v.dtype),
            pltpu.VMEM((H * Dh // 128, 128), f32),
            pltpu.VMEM((W // 128, 8, 128), f32),
            pltpu.VMEM((16, D // 8 * 128), bf16),
            pltpu.VMEM((16, 128), f32),
            pltpu.SemaphoreType.DMA((2, NBUF)),
            pltpu.SemaphoreType.DMA((6,)),
            pltpu.SemaphoreType.DMA((len(DOWN_GROUPS),)),
        ],
        compiler_params=pltpu.CompilerParams(
            vmem_limit_bytes=100 * 2**20,
            disable_bounds_checks=True,
            disable_semaphore_checks=True,
        ),
    )(A_x, k, v, wq, wo, B_w_r, wg, wu, wd)
```

```python
import jax
import jax.numpy as jnp
from jax import lax
import jax.experimental.pallas as pl
import jax.experimental.pallas.tpu as pltpu

EPS = 1e-5
BLK = 128
RUN = 64
NBUF = 3
KV_PAIR = 2
KV_STEP = 7
GAP_ATTN, GAP_FFN = 480, 240
DOWN_MXU, DOWN_VPU = (32, 20), (6, 2)
QUEUE_LAG = 24

f32, bf16 = jnp.float32, jnp.bfloat16


def _tile_order(w, rows):
    r, c = w.shape
    return w.reshape(r // 8, 8, c // 128, 128).transpose(0, 2, 1, 3).reshape(-1, rows, 128)


def _layernorm(x):
    m = jnp.mean(x, axis=-1, keepdims=True)
    d = x - m
    v = jnp.mean(d * d, axis=-1, keepdims=True)
    return d / jnp.sqrt(v + EPS)


def _kernel(x_hbm, k_hbm, v_hbm, wq_hbm, wo_hbm, wr_hbm, wg_hbm, wu_hbm, wd_hbm,
            o_ref,
            x_s, wr_s, wq_s, wo_s, wg_s, wu_s, wd_s, k_s, v_s, q_s, p_s, lhs_s, y_s, col_s,
            sem_kv, sem_w, sem_d, *, H, Dh, Sk, W, F):
    D = x_hbm.shape[-1]
    TR = Dh // 8
    HALVES = W // (16 * 128)
    DT, FT = D // 128, F // 128
    QG = H * Dh // (16 * 128)

    def copy(src, src_at, src_row, dst, dst_at, dst_row, sem, queue):
        def runs(ref, at, row):
            row = row if isinstance(row, int) else pl.multiple_of(row, RUN)
            return ref.at[pl.ds(at, 2), pl.ds(row, RUN)]
        pltpu.make_async_copy(runs(src, src_at, src_row), runs(dst, dst_at, dst_row), sem).start(priority=queue)

    def done(dst, sem):
        pltpu.make_async_copy(dst, dst, sem).wait()

    def weights_start(jobs, lo, hi):
        pairs = jobs[0][0].shape[0] // 2
        per = 2 // len(jobs)

        def body(_, at):
            u, v = at
            for queue in range(2):
                src, dst, sem = jobs[queue % len(jobs)]
                copy(src, 2 * u, RUN * v, dst, 2 * u, RUN * v, sem, queue)
                if queue == 1 or per == 2:
                    wrap = u + 1 == pairs
                    u, v = jnp.where(wrap, 0, u + 1), jnp.where(wrap, v + 1, v)
            return u, v
        lax.fori_loop(lo // per, hi // per, body, (lo % pairs, lo // pairs))

    def kv_start(h, slot):
        for a, (src, dst) in enumerate(((k_hbm, k_s), (v_hbm, v_s))):
            for part in range(2 * HALVES):
                def body(_, pair):
                    for queue in range(2):
                        j = pair // KV_PAIR
                        e = pair - j * KV_PAIR
                        copy(src, h * (TR // KV_PAIR) + 2 * j, e * (Sk // 16) + (Sk - W) // 16 + RUN * part,
                             dst.at[slot, part // 2], 2 * j, e * BLK + RUN * (part % 2),
                             sem_kv.at[a, slot], queue)
                        pair = pair + KV_STEP
                        pair = jnp.where(pair >= TR // 2, pair - TR // 2, pair)
                    return pair
                lax.fori_loop(0, TR // 4, body, 0)

    n_attn = wq_hbm.shape[0] * wq_hbm.shape[1] // BLK
    n_ffn = wd_hbm.shape[0] * wd_hbm.shape[1] // BLK
    down_at = [(i % (wd_hbm.shape[0] // 2), i // (wd_hbm.shape[0] // 2)) for i in range(n_ffn)]
    landing = sorted(range(n_ffn), key=lambda i: i + QUEUE_LAG * (i % 2))
    down_tile = [2 * GAP_FFN * down_at[i][0] + 8 * down_at[i][1] + GAP_FFN * (t // 8) + t % 8
                 for i in landing for t in range(16)]
    groups = DOWN_MXU + DOWN_VPU
    bounds = [sum(groups[:g]) for g in range(len(groups) + 1)]

    def down_start():
        for i, (u, v) in enumerate(down_at):
            slot = landing.index(i)
            g = max(g for g in range(len(groups)) if bounds[g] <= slot)
            copy(wd_hbm, 2 * u, RUN * v, wd_s, 2 * slot, 0, sem_d.at[g], i % 2)

    x_cp = pltpu.make_async_copy(x_hbm, x_s, sem_w.at[0])
    wr_cp = pltpu.make_async_copy(wr_hbm, wr_s, sem_w.at[1])

    weights_start([(wq_hbm, wq_s, sem_w.at[2])], 0, n_attn)
    weights_start([(wo_hbm, wo_s, sem_w.at[3])], 0, n_attn)
    x_cp.start()
    wr_cp.start(priority=1)
    kv_start(0, 0)

    lane = lax.broadcasted_iota(jnp.int32, (8, 128), 1)
    row8 = lax.broadcasted_iota(jnp.int32, (8, 128), 0)
    lane16 = lax.broadcasted_iota(jnp.int32, (16, 128), 1)
    row16 = lax.broadcasted_iota(jnp.int32, (16, 128), 0)
    tile, tile16, in_tile = lane >> 3, lane16 >> 3, lane & 7
    diagonal = tile16 == row16

    def gather(vec, idx):
        return jnp.take_along_axis(jnp.broadcast_to(vec, (8, 128)), idx, axis=1)

    def spread(c, g, keep):
        lhs_s[:, c * 128:(c + 1) * 128] = jnp.where(keep, jnp.concatenate([g, g], axis=0), 0.0).astype(bf16)

    def matmul(lo, hi, w):
        return jnp.dot(lhs_s[:, lo * 128:hi * 128], w.reshape(-1, 128), preferred_element_type=f32)

    x_cp.wait()
    x = x_s[0].astype(f32)
    xn = _layernorm(x)
    for tr in range(D // 8):
        spread(tr, gather(xn[:, tr // 16 * 128:(tr // 16 + 1) * 128], in_tile + 8 * (tr % 16)), diagonal)
    done(wq_s, sem_w.at[2])
    for g in range(QG):
        at = [divmod((QG * tr + g) * BLK, wq_s.shape[1]) for tr in range(D // 8)]
        w = jnp.concatenate([wq_s[a, r:r + BLK, :] for a, r in at], axis=0)
        q_s[16 * g:16 * (g + 1)] = matmul(0, D // 8, w)
    kv_start(1, 1)
    done(wo_s, sem_w.at[3])

    scale = Dh ** -0.5
    heads_per_gap = wo_s.shape[1] // (Dh * DT)

    def head(h, slot, acc):
        for tr in range(TR):
            f = h * Dh + 8 * tr
            spread(tr, gather(q_s[pl.ds(f >> 7, 1), :], in_tile + (f & 127)), diagonal)
        done(k_s.at[slot], sem_kv.at[0, slot])
        s = jnp.concatenate([matmul(0, TR, k_s[slot, hf]) for hf in range(HALVES)], axis=0) * scale
        m = jnp.max(jnp.max(s, axis=0, keepdims=True), axis=1, keepdims=True)
        e = jnp.exp(s - m)
        inv = 1.0 / jnp.sum(jnp.sum(e, axis=0, keepdims=True), axis=1, keepdims=True)
        for j in range(W // 128):
            p_s[j] = jnp.broadcast_to(e[j:j + 1], (8, 128))
        done(v_s.at[slot], sem_kv.at[1, slot])
        acc = list(acc)
        for t2 in range(TR // 2):
            o = []
            for tr in (2 * t2, 2 * t2 + 1):
                a0 = jnp.zeros((8, 128), f32)
                a1 = jnp.zeros((8, 128), f32)
                for hf in range(HALVES):
                    for j in range(0, 16, 2):
                        r = tr % KV_PAIR * BLK + 8 * j
                        vv = v_s[slot, hf, tr // KV_PAIR, r:r + 16, :].astype(f32)
                        a0 = a0 + vv[:8] * p_s[hf * 16 + j]
                        a1 = a1 + vv[8:] * p_s[hf * 16 + j + 1]
                o.append(jnp.sum(a0 + a1, axis=-1, keepdims=True) * inv)
            row = pl.multiple_of(h % heads_per_gap * (Dh * DT) + t2 * 16 * DT, 16)
            ww = wo_s[h // heads_per_gap, pl.ds(row, 16 * DT), :].astype(f32)
            for t in range(2 * DT):
                acc[t % DT] = acc[t % DT] + ww[8 * t:8 * t + 8] * o[t // DT]
        return tuple(acc)

    def step(h, carry):
        slot, acc = carry

        @pl.when(h < H - 2)
        def _():
            kv_start(h + 2, jnp.where(slot + 2 >= NBUF, slot + 2 - NBUF, slot + 2))

        for part in range(2):
            @pl.when(h == H - 2 + part)
            def _():
                weights_start([(wg_hbm, wg_s, sem_w.at[4]), (wu_hbm, wu_s, sem_w.at[5])],
                              n_ffn // 2 * part, n_ffn // 2 * (part + 1))
        return jnp.where(slot + 1 == NBUF, 0, slot + 1), head(h, slot, acc)

    acc = tuple(jnp.zeros((8, 128), f32) for _ in range(DT))
    _, acc = lax.fori_loop(0, H, step, (0, acc))
    down_start()

    hres = x + jnp.concatenate([jnp.sum(a, axis=0, keepdims=True) for a in acc], axis=1)
    hn = _layernorm(hres)
    wr_cp.wait()
    wr = wr_s[...].astype(f32).reshape(1, D)
    gate = jax.nn.sigmoid(jnp.sum(hn * wr, axis=-1, keepdims=True))
    resid = hres + hn

    def spread_tiles(c, tiles, vec, ct):
        g = keep = None
        for j in range(16):
            if j and tiles[j] == tiles[j - 1] + 1 and tiles[j] % (16 * ct):
                continue
            i, r = divmod(tiles[j], 16 * ct)
            g_new = gather(vec(i), (8 * ((tile + (r - j + 16 * ct)) // ct) + in_tile) & 127)
            keep_new = (tile16 + (r - j + 16 * ct)) % ct == row16
            g = g_new if j == 0 else jnp.where(tile >= j, g_new, g)
            keep = keep_new if j == 0 else (keep_new & (tile16 >= j)) | (keep & (tile16 < j))
        spread(c, g, keep)

    for c in range(n_ffn):
        spread_tiles(c, range(16 * c, 16 * c + 16), lambda i: hn[:, 128 * i:128 * (i + 1)], FT)
    done(wg_s, sem_w.at[4])
    g = matmul(0, n_ffn, wg_s[...])
    y_s[...] = g * jax.nn.sigmoid(g)
    done(wu_s, sem_w.at[5])
    gu = y_s[...] * matmul(0, n_ffn, wu_s[...])

    n_mxu = sum(DOWN_MXU)
    for c in range(n_mxu):
        spread_tiles(c, down_tile[16 * c:16 * c + 16], lambda i: gu[i:i + 1], DT)
    last_rows = sorted({t // DT for t in down_tile[16 * n_mxu:]})
    for n, tr in enumerate(last_rows):
        col_s[n] = gather(gu[tr // 16:tr // 16 + 1], row8 + 8 * (tr % 16))
    y_s[...] = jnp.zeros_like(y_s)
    z = [[] for _ in range(DT)]
    for g in range(len(groups)):
        lo, hi = bounds[g], bounds[g + 1]
        done(wd_s.at[2 * lo:2 * hi], sem_d.at[g])
        if g < len(DOWN_MXU):
            y_s[...] = y_s[...] + matmul(lo, hi, wd_s[2 * lo:2 * hi])
            continue
        for t in range(16 * lo, 16 * hi, 2):
            ww = wd_s[t // 8, 8 * (t % 8):8 * (t % 8) + 16, :].astype(f32)
            for u in range(2):
                tr, tc = divmod(down_tile[t + u], DT)
                term = ww[8 * u:8 * u + 8] * col_s[last_rows.index(tr)]
                z[tc] = [z[tc][0] + term if z[tc] else term]
    y = y_s[...]
    y = jnp.concatenate([y[i:i + 1] + jnp.sum(z[i][0], axis=0, keepdims=True) for i in range(DT)], axis=1)
    o_ref[0] = (resid + y * gate).astype(o_ref.dtype)


@jax.jit
def pallas_sequential_preLN__sliding_block_cached__moe_arch_mod__decode_kernel(
    A_x: jax.Array,
    A_k_cache: jax.Array,
    A_v_cache: jax.Array,
    A_wq: jax.Array,
    A_wo: jax.Array,
    B_x: jax.Array,
    B_w_r: jax.Array,
    B_w_gate: jax.Array,
    B_w_up: jax.Array,
    B_w_down: jax.Array,
):
    del B_x
    _, H, Sk, Dh = A_k_cache.shape
    D, F = B_w_gate.shape
    W = min(4096, max(256, Sk // 4))
    k, v = (_tile_order(jnp.transpose(c, (0, 1, 3, 2)).reshape(H * Dh, Sk), KV_PAIR * Sk // 16)
            for c in (A_k_cache, A_v_cache))
    wq, wo = (_tile_order(w, 8 * GAP_ATTN) for w in (A_wq, A_wo))
    wg, wu, wd = (_tile_order(w, 8 * GAP_FFN) for w in (B_w_gate, B_w_up, B_w_down))
    ring = (NBUF, W // (16 * 128), Dh // (8 * KV_PAIR), KV_PAIR * BLK, 128)

    def like(a):
        return pltpu.VMEM(a.shape, a.dtype)

    def kernel(*refs):
        _kernel(*refs, H=H, Dh=Dh, Sk=Sk, W=W, F=F)

    return pl.pallas_call(
        kernel,
        out_shape=jax.ShapeDtypeStruct(A_x.shape, A_x.dtype),
        in_specs=[pl.BlockSpec(memory_space=pl.ANY)] * 9,
        scratch_shapes=[
            like(A_x), like(B_w_r), like(wq), like(wo), like(wg), like(wu),
            pltpu.VMEM((F * D // (128 * RUN), RUN, 128), wd.dtype),
            pltpu.VMEM(ring, k.dtype),
            pltpu.VMEM(ring, v.dtype),
            pltpu.VMEM((H * Dh // 128, 128), f32),
            pltpu.VMEM((W // 128, 8, 128), f32),
            pltpu.VMEM((16, D // 8 * 128), bf16),
            pltpu.VMEM((16, 128), f32),
            pltpu.VMEM((6 * sum(DOWN_VPU), 8, 128), f32),
            pltpu.SemaphoreType.DMA((2, NBUF)),
            pltpu.SemaphoreType.DMA((6,)),
            pltpu.SemaphoreType.DMA((len(DOWN_MXU + DOWN_VPU),)),
        ],
        compiler_params=pltpu.CompilerParams(
            vmem_limit_bytes=100 * 2**20,
            disable_bounds_checks=True,
            disable_semaphore_checks=True,
        ),
    )(A_x, k, v, wq, wo, B_w_r, wg, wu, wd)
```

```python
import jax
import jax.numpy as jnp
from jax import lax
import jax.experimental.pallas as pl
import jax.experimental.pallas.tpu as pltpu

EPS = 1e-5
BLK = 128
RUN = 64
NBUF = 3
KV_PAIR = 2
KV_STEP = 7
GAP_ATTN, GAP_FFN = 480, 240
DOWN_MXU, DOWN_VPU = (36, 16), (6, 2)
BACKLOG = 12

f32, bf16 = jnp.float32, jnp.bfloat16


def _tile_order(w, rows):
    r, c = w.shape
    return w.reshape(r // 8, 8, c // 128, 128).transpose(0, 2, 1, 3).reshape(-1, rows, 128)


def _layernorm(x):
    m = jnp.mean(x, axis=-1, keepdims=True)
    d = x - m
    v = jnp.mean(d * d, axis=-1, keepdims=True)
    return d / jnp.sqrt(v + EPS)


def _kernel(x_hbm, k_hbm, v_hbm, wq_hbm, wo_hbm, wr_hbm, wg_hbm, wu_hbm, wd_hbm,
            o_ref,
            x_s, wr_s, wq_s, wo_s, wg_s, wu_s, wd_s, k_s, v_s, q_s, p_s, lhs_s, y_s, col_s,
            sem_kv, sem_w, sem_d, *, H, Dh, Sk, W, F):
    D = x_hbm.shape[-1]
    TR = Dh // 8
    HALVES = W // (16 * 128)
    DT, FT = D // 128, F // 128
    QG = H * Dh // (16 * 128)

    def copy(src, src_at, src_row, dst, dst_at, dst_row, sem, queue):
        def runs(ref, at, row):
            row = row if isinstance(row, int) else pl.multiple_of(row, RUN)
            return ref.at[pl.ds(at, 2), pl.ds(row, RUN)]
        pltpu.make_async_copy(runs(src, src_at, src_row), runs(dst, dst_at, dst_row), sem).start(priority=queue)

    def done(dst, sem):
        pltpu.make_async_copy(dst, dst, sem).wait()

    def weights_start(jobs, lo, hi):
        pairs = jobs[0][0].shape[0] // 2
        per = 2 // len(jobs)

        def body(_, at):
            u, v = at
            for queue in range(2):
                src, dst, sem = jobs[queue % len(jobs)]
                copy(src, 2 * u, RUN * v, dst, 2 * u, RUN * v, sem, queue)
                if queue == 1 or per == 2:
                    wrap = u + 1 == pairs
                    u, v = jnp.where(wrap, 0, u + 1), jnp.where(wrap, v + 1, v)
            return u, v
        lax.fori_loop(lo // per, hi // per, body, (lo % pairs, lo // pairs))

    def kv_start(h, slot):
        for a, (src, dst) in enumerate(((k_hbm, k_s), (v_hbm, v_s))):
            for part in range(2 * HALVES):
                def body(_, pair):
                    for queue in range(2):
                        j = pair // KV_PAIR
                        e = pair - j * KV_PAIR
                        copy(src, h * (TR // KV_PAIR) + 2 * j, e * (Sk // 16) + (Sk - W) // 16 + RUN * part,
                             dst.at[slot, part // 2], 2 * j, e * BLK + RUN * (part % 2),
                             sem_kv.at[a, slot], queue)
                        pair = pair + KV_STEP
                        pair = jnp.where(pair >= TR // 2, pair - TR // 2, pair)
                    return pair
                lax.fori_loop(0, TR // 4, body, 0)

    n_attn = wq_hbm.shape[0] * wq_hbm.shape[1] // BLK
    n_ffn = wd_hbm.shape[0] * wd_hbm.shape[1] // BLK
    down_at = [(i % (wd_hbm.shape[0] // 2), i // (wd_hbm.shape[0] // 2)) for i in range(n_ffn)]
    landing = list(range(BACKLOG)) + sorted(range(BACKLOG, n_ffn), key=lambda i: i + 2 * BACKLOG * (i % 2))
    down_tile = [2 * GAP_FFN * down_at[i][0] + 8 * down_at[i][1] + GAP_FFN * (t // 8) + t % 8
                 for i in landing for t in range(16)]
    groups = DOWN_MXU + DOWN_VPU
    bounds = [sum(groups[:g]) for g in range(len(groups) + 1)]

    up_jobs = [(wg_hbm, wg_s, sem_w.at[4]), (wu_hbm, wu_s, sem_w.at[5])]
    n_paired = n_ffn - BACKLOG // 2

    def down_start():
        pairs = wd_hbm.shape[0] // 2
        for n, (src, dst, sem) in enumerate(up_jobs):
            def body(j, _):
                c, i = n_paired + j, n * (BACKLOG // 2) + j
                copy(src, 2 * (c % pairs), RUN * (c // pairs), dst, 2 * (c % pairs), RUN * (c // pairs), sem, 0)
                copy(wd_hbm, 2 * (i % pairs), RUN * (i // pairs), wd_s, 2 * i, 0, sem_d.at[0], 1)
            lax.fori_loop(0, BACKLOG // 2, body, None)
        for i in range(BACKLOG, n_ffn):
            u, v = down_at[i]
            slot = landing.index(i)
            g = max(g for g in range(len(groups)) if bounds[g] <= slot)
            copy(wd_hbm, 2 * u, RUN * v, wd_s, 2 * slot, 0, sem_d.at[g], i % 2)

    x_cp = pltpu.make_async_copy(x_hbm, x_s, sem_w.at[0])
    wr_cp = pltpu.make_async_copy(wr_hbm, wr_s, sem_w.at[1])

    for i in range(BACKLOG):
        u, v = i % (wq_hbm.shape[0] // 2), i // (wq_hbm.shape[0] // 2)
        copy(wq_hbm, 2 * u, RUN * v, wq_s, 2 * u, RUN * v, sem_w.at[2], 1)
    weights_start([(wq_hbm, wq_s, sem_w.at[2])], BACKLOG, n_attn)
    weights_start([(wo_hbm, wo_s, sem_w.at[3])], 0, n_attn)
    x_cp.start()
    wr_cp.start(priority=1)
    kv_start(0, 0)

    lane = lax.broadcasted_iota(jnp.int32, (8, 128), 1)
    row8 = lax.broadcasted_iota(jnp.int32, (8, 128), 0)
    lane16 = lax.broadcasted_iota(jnp.int32, (16, 128), 1)
    row16 = lax.broadcasted_iota(jnp.int32, (16, 128), 0)
    tile, tile16, in_tile = lane >> 3, lane16 >> 3, lane & 7
    diagonal = tile16 == row16

    def gather(vec, idx):
        return jnp.take_along_axis(jnp.broadcast_to(vec, (8, 128)), idx, axis=1)

    def spread(c, g, keep):
        lhs_s[:, c * 128:(c + 1) * 128] = jnp.where(keep, jnp.concatenate([g, g], axis=0), 0.0).astype(bf16)

    def matmul(lo, hi, w):
        return jnp.dot(lhs_s[:, lo * 128:hi * 128], w.reshape(-1, 128), preferred_element_type=f32)

    x_cp.wait()
    x = x_s[0].astype(f32)
    xn = _layernorm(x)
    for tr in range(D // 8):
        spread(tr, gather(xn[:, tr // 16 * 128:(tr // 16 + 1) * 128], in_tile + 8 * (tr % 16)), diagonal)
    done(wq_s, sem_w.at[2])
    for g in range(QG):
        at = [divmod((QG * tr + g) * BLK, wq_s.shape[1]) for tr in range(D // 8)]
        w = jnp.concatenate([wq_s[a, r:r + BLK, :] for a, r in at], axis=0)
        q_s[16 * g:16 * (g + 1)] = matmul(0, D // 8, w)
    kv_start(1, 1)
    done(wo_s, sem_w.at[3])

    scale = Dh ** -0.5
    heads_per_gap = wo_s.shape[1] // (Dh * DT)

    def head(h, slot, acc):
        for tr in range(TR):
            f = h * Dh + 8 * tr
            spread(tr, gather(q_s[pl.ds(f >> 7, 1), :], in_tile + (f & 127)), diagonal)
        done(k_s.at[slot], sem_kv.at[0, slot])
        s = jnp.concatenate([matmul(0, TR, k_s[slot, hf]) for hf in range(HALVES)], axis=0) * scale
        m = jnp.max(jnp.max(s, axis=0, keepdims=True), axis=1, keepdims=True)
        e = jnp.exp(s - m)
        inv = 1.0 / jnp.sum(jnp.sum(e, axis=0, keepdims=True), axis=1, keepdims=True)
        for j in range(W // 128):
            p_s[j] = jnp.broadcast_to(e[j:j + 1], (8, 128))
        done(v_s.at[slot], sem_kv.at[1, slot])
        acc = list(acc)
        for t2 in range(TR // 2):
            o = []
            for tr in (2 * t2, 2 * t2 + 1):
                a0 = jnp.zeros((8, 128), f32)
                a1 = jnp.zeros((8, 128), f32)
                for hf in range(HALVES):
                    for j in range(0, 16, 2):
                        r = tr % KV_PAIR * BLK + 8 * j
                        vv = v_s[slot, hf, tr // KV_PAIR, r:r + 16, :].astype(f32)
                        a0 = a0 + vv[:8] * p_s[hf * 16 + j]
                        a1 = a1 + vv[8:] * p_s[hf * 16 + j + 1]
                o.append(jnp.sum(a0 + a1, axis=-1, keepdims=True) * inv)
            row = pl.multiple_of(h % heads_per_gap * (Dh * DT) + t2 * 16 * DT, 16)
            ww = wo_s[h // heads_per_gap, pl.ds(row, 16 * DT), :].astype(f32)
            for t in range(2 * DT):
                acc[t % DT] = acc[t % DT] + ww[8 * t:8 * t + 8] * o[t // DT]
        return tuple(acc)

    def step(h, carry):
        slot, acc = carry

        @pl.when(h < H - 2)
        def _():
            kv_start(h + 2, jnp.where(slot + 2 >= NBUF, slot + 2 - NBUF, slot + 2))

        for part in range(2):
            @pl.when(h == H - 2 + part)
            def _():
                weights_start(up_jobs, n_paired * part // 2, n_paired * (part + 1) // 2)
        return jnp.where(slot + 1 == NBUF, 0, slot + 1), head(h, slot, acc)

    acc = tuple(jnp.zeros((8, 128), f32) for _ in range(DT))
    _, acc = lax.fori_loop(0, H, step, (0, acc))
    down_start()

    hres = x + jnp.concatenate([jnp.sum(a, axis=0, keepdims=True) for a in acc], axis=1)
    hn = _layernorm(hres)
    wr_cp.wait()
    wr = wr_s[...].astype(f32).reshape(1, D)
    gate = jax.nn.sigmoid(jnp.sum(hn * wr, axis=-1, keepdims=True))
    resid = hres + hn

    def spread_tiles(c, tiles, vec, ct):
        g = keep = None
        for j in range(16):
            if j and tiles[j] == tiles[j - 1] + 1 and tiles[j] % (16 * ct):
                continue
            i, r = divmod(tiles[j], 16 * ct)
            g_new = gather(vec(i), (8 * ((tile + (r - j + 16 * ct)) // ct) + in_tile) & 127)
            keep_new = (tile16 + (r - j + 16 * ct)) % ct == row16
            g = g_new if j == 0 else jnp.where(tile >= j, g_new, g)
            keep = keep_new if j == 0 else (keep_new & (tile16 >= j)) | (keep & (tile16 < j))
        spread(c, g, keep)

    for c in range(n_ffn):
        spread_tiles(c, range(16 * c, 16 * c + 16), lambda i: hn[:, 128 * i:128 * (i + 1)], FT)
    done(wg_s, sem_w.at[4])
    g = matmul(0, n_ffn, wg_s[...])
    y_s[...] = g * jax.nn.sigmoid(g)
    done(wu_s, sem_w.at[5])
    gu = y_s[...] * matmul(0, n_ffn, wu_s[...])

    n_mxu = sum(DOWN_MXU)
    for c in range(n_mxu):
        spread_tiles(c, down_tile[16 * c:16 * c + 16], lambda i: gu[i:i + 1], DT)
    last_rows = sorted({t // DT for t in down_tile[16 * n_mxu:]})
    for n, tr in enumerate(last_rows):
        col_s[n] = gather(gu[tr // 16:tr // 16 + 1], row8 + 8 * (tr % 16))
    y_s[...] = jnp.zeros_like(y_s)
    z = [[] for _ in range(DT)]
    for g in range(len(groups)):
        lo, hi = bounds[g], bounds[g + 1]
        done(wd_s.at[2 * lo:2 * hi], sem_d.at[g])
        if g < len(DOWN_MXU):
            y_s[...] = y_s[...] + matmul(lo, hi, wd_s[2 * lo:2 * hi])
            continue
        for t in range(16 * lo, 16 * hi, 2):
            ww = wd_s[t // 8, 8 * (t % 8):8 * (t % 8) + 16, :].astype(f32)
            for u in range(2):
                tr, tc = divmod(down_tile[t + u], DT)
                term = ww[8 * u:8 * u + 8] * col_s[last_rows.index(tr)]
                z[tc] = [z[tc][0] + term if z[tc] else term]
    y = y_s[...]
    y = jnp.concatenate([y[i:i + 1] + jnp.sum(z[i][0], axis=0, keepdims=True) for i in range(DT)], axis=1)
    o_ref[0] = (resid + y * gate).astype(o_ref.dtype)


@jax.jit
def pallas_sequential_preLN__sliding_block_cached__moe_arch_mod__decode_kernel(
    A_x: jax.Array,
    A_k_cache: jax.Array,
    A_v_cache: jax.Array,
    A_wq: jax.Array,
    A_wo: jax.Array,
    B_x: jax.Array,
    B_w_r: jax.Array,
    B_w_gate: jax.Array,
    B_w_up: jax.Array,
    B_w_down: jax.Array,
):
    del B_x
    _, H, Sk, Dh = A_k_cache.shape
    D, F = B_w_gate.shape
    W = min(4096, max(256, Sk // 4))
    k, v = (_tile_order(jnp.transpose(c, (0, 1, 3, 2)).reshape(H * Dh, Sk), KV_PAIR * Sk // 16)
            for c in (A_k_cache, A_v_cache))
    wq, wo = (_tile_order(w, 8 * GAP_ATTN) for w in (A_wq, A_wo))
    wg, wu, wd = (_tile_order(w, 8 * GAP_FFN) for w in (B_w_gate, B_w_up, B_w_down))
    ring = (NBUF, W // (16 * 128), Dh // (8 * KV_PAIR), KV_PAIR * BLK, 128)

    def like(a):
        return pltpu.VMEM(a.shape, a.dtype)

    def kernel(*refs):
        _kernel(*refs, H=H, Dh=Dh, Sk=Sk, W=W, F=F)

    return pl.pallas_call(
        kernel,
        out_shape=jax.ShapeDtypeStruct(A_x.shape, A_x.dtype),
        in_specs=[pl.BlockSpec(memory_space=pl.ANY)] * 9,
        scratch_shapes=[
            like(A_x), like(B_w_r), like(wq), like(wo), like(wg), like(wu),
            pltpu.VMEM((F * D // (128 * RUN), RUN, 128), wd.dtype),
            pltpu.VMEM(ring, k.dtype),
            pltpu.VMEM(ring, v.dtype),
            pltpu.VMEM((H * Dh // 128, 128), f32),
            pltpu.VMEM((W // 128, 8, 128), f32),
            pltpu.VMEM((16, D // 8 * 128), bf16),
            pltpu.VMEM((16, 128), f32),
            pltpu.VMEM((6 * sum(DOWN_VPU), 8, 128), f32),
            pltpu.SemaphoreType.DMA((2, NBUF)),
            pltpu.SemaphoreType.DMA((6,)),
            pltpu.SemaphoreType.DMA((len(DOWN_MXU + DOWN_VPU),)),
        ],
        compiler_params=pltpu.CompilerParams(
            vmem_limit_bytes=64 * 2**20,
            disable_bounds_checks=True,
            disable_semaphore_checks=True,
        ),
    )(A_x, k, v, wq, wo, B_w_r, wg, wu, wd)
```
